```python
import os as _os
_os.environ.setdefault("JAX_PLATFORMS", "cpu")
import jax
import jax.numpy as jnp

def _softmax(x, axis=-1):
    return jax.nn.softmax(x, axis=axis)
def _gelu(x):
    return jax.nn.gelu(x, approximate=True)
def _silu(x):
    return jax.nn.silu(x)
def _sigmoid(x):
    return jax.nn.sigmoid(x)
def _layernorm(x, axis=-1, eps=1e-5):
    m = jnp.mean(x, axis=axis, keepdims=True)
    v = jnp.var(x, axis=axis, keepdims=True)
    return (x - m) / jnp.sqrt(v + eps)
def _scatter_add(tgt, idx, src, axis=0):
    return tgt.at[idx].add(src)
def _segment_sum(src, seg, n):
    return jax.ops.segment_sum(src, seg, n)
class _Rng:
    def __init__(self, key):
        self._k = key
    def _next(self):
        self._k, sub = jax.random.split(self._k)
        return sub
    def normal(self, shape):
        return jax.random.normal(self._next(), shape, dtype=jnp.bfloat16)
    def randint(self, lo, hi, shape):
        return jax.random.randint(self._next(), shape, lo, hi, dtype=jnp.int32)
    def uniform(self, shape, lo=0.0, hi=1.0):
        return jax.random.uniform(self._next(), shape, jnp.bfloat16, lo, hi)
    def permutation(self, n):
        return jax.random.permutation(self._next(), n)


kernel_name = 'parallel_sum__sliding_local_dilated__glu_gated_geglu__prompt'

def setup_inputs():
    _rng = _Rng(jax.random.key(int.from_bytes(__import__("os").urandom(4), "little")))
    _w = (lambda a: (lambda t: t.astype(jnp.bfloat16) if jnp.issubdtype(t.dtype, jnp.floating) else t)(jnp.asarray(a)))
    def _A_setup():
        B, S, D = 1, 2048, 512
        return {
            "x": _w((lambda *s: _rng.normal(s) * 0.05)(B, S, D)),
            "wqkv": _w((lambda *s: _rng.normal(s) * 0.05)(D, 3 * D)),
            "wo": _w((lambda *s: _rng.normal(s) * 0.05)(D, D)),
        }
    _A_in = _A_setup()

    def _B_setup():
        B, S, Dm, Df = 1, 2048, 512, 1376
        return {
            "x": _w((lambda *s: _rng.normal(s) * 0.05)(B, S, Dm)),
            "w_gate": _w((lambda *s: _rng.normal(s) * 0.1)(Dm, Df) * (Dm ** -0.5)),
            "w_up": _w((lambda *s: _rng.normal(s) * 0.1)(Dm, Df) * (Dm ** -0.5)),
            "w_down": _w((lambda *s: _rng.normal(s) * 0.1)(Df, Dm) * (Df ** -0.5)),
        }
    _B_in = _B_setup()

    return {
        "A_x": _A_in["x"],
        "A_wqkv": _A_in["wqkv"],
        "A_wo": _A_in["wo"],
        "B_x": _B_in["x"],
        "B_w_gate": _B_in["w_gate"],
        "B_w_up": _B_in["w_up"],
        "B_w_down": _B_in["w_down"],
    }

def reference(A_x, A_wqkv, A_wo, B_x, B_w_gate, B_w_up, B_w_down):
    def _A_ref(x, wqkv, wo):
        B, S, D = x.shape
        H = 32; Dh = D // H
        W, dil = 8, 2
        qkv = (lambda x, *d: x.transpose(*d))((x @ wqkv).reshape(B, S, 3, H, Dh), 2, 0, 3, 1, 4)
        q, k, v = qkv[0], qkv[1], qkv[2]
        scale = Dh ** -0.5
        pos = jnp.arange(S)
        off = jnp.arange(W) * dil
        idx = pos[:, None] - off[None, :]
        mask = idx >= 0
        idx_c = jnp.where(mask, idx, 0).reshape(-1)
        kg = k[:, :, idx_c, :].reshape(B, H, S, W, Dh)
        vg = v[:, :, idx_c, :].reshape(B, H, S, W, Dh)
        logits = jnp.einsum("bhsd,bhswd->bhsw", q, kg) * scale
        logits = jnp.where(mask[None, None, :, :], logits, -1e9)
        attn = _softmax(logits, axis=-1)
        o = jnp.einsum("bhsw,bhswd->bhsd", attn, vg)
        return (lambda x, *d: x.transpose(*d))(o, 0, 2, 1, 3).reshape(B, S, D) @ wo

    def _B_ref(x, w_gate, w_up, w_down):
        g = jnp.einsum("bsd,df->bsf", x, w_gate)
        u = jnp.einsum("bsd,df->bsf", x, w_up)
        h = _gelu(g) * u
        return jnp.einsum("bsf,fd->bsd", h, w_down)

    x = A_x
    xn = _layernorm(x, axis=-1)
    return x + _A_ref(xn, A_wqkv, A_wo) + _B_ref(xn, B_w_gate, B_w_up, B_w_down)
```

```python
import contextlib
import jax
import jax.numpy as jnp
import numpy as np
from jax import lax
import jax.experimental.pallas as pl
import jax.experimental.pallas.tpu as pltpu

S, D, H, DH, W, DIL, DF = 2048, 512, 32, 16, 8, 2, 1376
M = 256
NB = S // M
HALO = 16
LOG2E = 1.4426950408889634
NT = (((1,), (1,)), ((), ()))
U32 = int(1)
NODMA = int(0)
SCOPES = int(0)
FLAGS = {k: True for k in 'XLA_TPU_RESCHEDULE_DMA_DONES'.split(",") if k} or None
GATED = int(1)
RG = int(8)
CH1 = [0, 256, 512, 768, 1024, 1376]
KCH = [0, 256, 512, 768, 1024, 1376]
UN = 128
bf = jnp.bfloat16
f32 = jnp.float32
u32 = jnp.uint32


def scope(name):
    return jax.named_scope(name) if SCOPES else contextlib.nullcontext()


class Buf:
    def __init__(self, ref):
        self.ref = ref
        self.packed = ref.dtype == u32

    def ld(self, r0, r1, c0, c1):
        if self.packed:
            return pltpu.bitcast(self.ref[r0 // 2:r1 // 2, c0:c1], bf)
        return self.ref[r0:r1, c0:c1]

    def st(self, r0, r1, c0, c1, val):
        if self.packed:
            self.ref[r0 // 2:r1 // 2, c0:c1] = pltpu.bitcast(val, u32)
        else:
            self.ref[r0:r1, c0:c1] = val


def _perm_tile_cols(wu, j):
    rows = wu.shape[0]
    lane = lax.broadcasted_iota(jnp.int32, (rows, 128), 1)
    hh = lane & 31
    src_tile = hh >> 3
    idx = (hh & 7) * 16 + 4 * j + (lane >> 5)
    acc = None
    for t in range(4):
        g = jnp.take_along_axis(wu[:, t * 128:(t + 1) * 128], idx, axis=1)
        acc = g if acc is None else jnp.where(src_tile == t, g, acc)
    return acc


NXU = S // UN
NWU = DF // UN
SX, SG, SU, SD = 0, NXU, NXU + NWU + 1, NXU + 2 * (NWU + 1)
SQ = NXU + 3 * (NWU + 1)
SO = SQ + 4
SOUT = SO + 1
NSEM = SOUT + NB


def _kernel(x_hbm, wqkv_hbm, wo_hbm, wg_hbm, wu_hbm, wd_hbm, out_hbm,
            x_v, wqkv_v, wo_v, wg_v, wu_v, wd_v, wg_p, wu_p, wd_p, xn_r, h_r, wqkvp_r, wop_r, wof,
            kbuf, vbuf, qbuf, o_r, out_v, sem):
    xn, hb, wqkvp, wop, ob = Buf(xn_r), Buf(h_r), Buf(wqkvp_r), Buf(wop_r), Buf(o_r)
    wgp, wup, wdp = Buf(wg_p), Buf(wu_p), Buf(wd_p)

    def unit(src, dst, base, i, rows=UN):
        sl = pl.ds(i * UN, rows) if isinstance(i, int) else pl.ds(pl.multiple_of(i * UN, UN), rows)
        return pltpu.make_async_copy(src.at[sl], dst.at[sl], sem.at[base + i])

    def start_units(src, dst, base, lo, hi):
        def body(i, c):
            unit(src, dst, base, i).start()
            return c
        lax.fori_loop(lo, hi, body, 0)

    def wait_units(src, dst, base, lo, hi, name):
        if NODMA:
            return
        with scope(name):
            for i in range(lo, hi):
                rows = UN if (i + 1) * UN <= src.shape[0] else src.shape[0] - i * UN
                unit(src, dst, base, i, rows).wait()

    def o_copy(i):
        return pltpu.make_async_copy(out_v.at[pl.ds(i * M, M)], out_hbm.at[pl.ds(i * M, M)], sem.at[SOUT + i])

    X = (x_hbm, x_v, SX)
    G = (wg_hbm, wg_v, SG)
    Uu = (wu_hbm, wu_v, SU)
    Dd = (wd_hbm, wd_v, SD)
    Q = (wqkv_hbm, wqkv_v, SQ)
    wo_copy = pltpu.make_async_copy(wo_hbm, wo_v, sem.at[SO])
    TAIL = DF - NWU * UN
    if not NODMA:
        start_units(*X, 0, 2)
        start_units(*G, 0, 2)
        start_units(*Uu, 0, 2)
        start_units(*X, 2, NXU)
        start_units(*G, 2, 6)
        start_units(*Uu, 2, 6)
        start_units(*G, 6, NWU)
        unit(*G, NWU, TAIL).start()
        start_units(*Uu, 6, NWU)
        unit(*Uu, NWU, TAIL).start()
        start_units(*Q, 0, 4)
        wo_copy.start()
        start_units(*Dd, 0, NWU)
        unit(*Dd, NWU, TAIL).start()

    kbuf[:, 0:HALO, :] = jnp.zeros((4, HALO, 128), f32)

    def ln(i):
        wait_units(*X, 2 * i, 2 * i + 2, f"waitx{i}")
        x = x_v[i * M:(i + 1) * M, :].astype(f32)
        mu = jnp.mean(x, axis=-1, keepdims=True)
        xc = x - mu
        var = jnp.mean(xc * xc, axis=-1, keepdims=True)
        v = (xc * lax.rsqrt(var + 1e-5)).astype(bf)
        xn.st(i * M, (i + 1) * M, 0, D, v)
        return v

    def getw(raw, pk, i, lo, hi):
        if not U32:
            return raw[lo:hi, :]
        if i == 0:
            v = raw[lo:hi, :]
            pk.st(lo, hi, 0, D, v)
            return v
        return pk.ld(lo, hi, 0, D)

    def gate_up(i, c, xv):
        lo, hi = CH1[c], CH1[c + 1]
        if i == 0:
            wait_units(*G, lo // UN, -(-hi // UN), f"waitg{c}")
        g = lax.dot_general(xv, getw(wg_v, wgp, i, lo, hi), NT, preferred_element_type=f32)
        if i == 0:
            wait_units(*Uu, lo // UN, -(-hi // UN), f"waitu{c}")
        u = lax.dot_general(xv, getw(wu_v, wup, i, lo, hi), NT, preferred_element_type=f32)
        hb.st(i * M, (i + 1) * M, lo, hi, (jax.nn.gelu(g, approximate=True) * u).astype(bf))

    def perm_qkv(t):
        wu = pltpu.bitcast(wqkv_v[:, t * 512:(t + 1) * 512], u32)
        for j in range(4):
            c0 = t * 512 + j * 128
            wqkvp.st(0, D, c0, c0 + 128, pltpu.bitcast(_perm_tile_cols(wu, j), bf))

    def perm_wo():
        for j in range(4):
            wof[j] = wo_v[:, j * 128:(j + 1) * 128].astype(f32)
        for d in range(DH):
            for j in range(4):
                wop.st(d * 32, (d + 1) * 32, j * 128, (j + 1) * 128, wof[j, pl.ds(d, 32, stride=16), :].astype(bf))

    def att(g0, R, gate):
        q = [qbuf[j, g0:g0 + R, :] for j in range(4)]
        if gate is not None:
            z = gate - gate
            z = jnp.concatenate([z] * (R // 8), axis=0) if R > 8 else z
            q = [qq + z for qq in q]
        ls = []
        for w in range(W):
            off = HALO + g0 - DIL * w
            s = None
            for j in range(4):
                p = q[j] * kbuf[j, off:off + R, :]
                s = p if s is None else s + p
            s = s + pltpu.roll(s, 64, 1)
            s = s + pltpu.roll(s, 32, 1)
            if g0 < DIL * w:
                pos = g0 + lax.broadcasted_iota(jnp.int32, (R, 128), 0)
                s = jnp.where(pos >= DIL * w, s, -1e9 * LOG2E)
            ls.append(s)
        m = ls[0]
        for w in range(1, W):
            m = jnp.maximum(m, ls[w])
        es = [jnp.exp2(l - m) for l in ls]
        den = es[0]
        for w in range(1, W):
            den = den + es[w]
        inv = pl.reciprocal(den, approx=True)
        inv = inv * (2.0 - den * inv)
        outs = []
        for j in range(4):
            o = None
            for w in range(W):
                off = HALO + g0 - DIL * w
                t = es[w] * vbuf[j, off:off + R, :]
                o = t if o is None else o + t
            outs.append(o * inv)
        return outs

    for c in range(len(CH1) - 1):
        for i in range(NB):
            xv = ln(i) if c == 0 else xn.ld(i * M, (i + 1) * M, 0, D)
            gate_up(i, c, xv)
        if c == 2:
            wait_units(*Q, 0, 4, "waitqkv")
            for t in range(3):
                perm_qkv(t)
        if c == 3:
            if not NODMA:
                with scope("waitwo"):
                    wo_copy.wait()
            perm_wo()
            wait_units(*Dd, 0, NWU + 1, "waitd")
            if U32:
                for lo in range(0, DF, UN):
                    hi = min(lo + UN, DF)
                    wdp.st(lo, hi, 0, D, wd_v[lo:hi, :])

    tnow = [0]
    milestones = []
    pending = []
    att_t0 = [int(v) for v in "3100,10000,17000,24000,31000,37300,43000,48700".split(",")]
    att_len = [int(v) for v in "6400,6400,6400,6400,5900,5300,5300,5300".split(",")]
    sched = []
    for i in range(NB):
        n = M // RG
        for c in range(n):
            sched.append((att_t0[i] + att_len[i] * c // n, i * M + c * RG))
    sidx = [0]
    q_done = [0]
    half = {}

    def emit_att(g0, gate):
        outs = att(g0, RG, gate)
        if RG % 16 == 0:
            for j in range(4):
                ob.st(g0, g0 + RG, j * 128, (j + 1) * 128, outs[j].astype(bf))
        else:
            if g0 % 16 == 0:
                half[0] = outs
            else:
                for j in range(4):
                    ob.st(g0 - 8, g0 + 8, j * 128, (j + 1) * 128,
                          jnp.concatenate([half[0][j], outs[j]], axis=0).astype(bf))

    def tick(cycles, val, nparts):
        for p in range(nparts):
            for hrow in range(2):
                t = tnow[0] + cycles * (2 * p + hrow) // (2 * nparts)
                gv = val[hrow * 128:hrow * 128 + 8, p * 128:(p + 1) * 128]
                while sidx[0] < len(sched) and sched[sidx[0]][0] <= t and sched[sidx[0]][1] < q_done[0] * M:
                    emit_att(sched[sidx[0]][1], gv if GATED else None)
                    sidx[0] += 1
        tnow[0] += cycles

    def qkv(i):
        r0 = i * M
        xv = xn.ld(r0, r0 + M, 0, D)
        for t, buf in ((1, kbuf), (2, vbuf), (0, qbuf)):
            y = jnp.dot(xv, wqkvp.ld(0, D, t * 512, (t + 1) * 512), preferred_element_type=f32)
            for j in range(4):
                yj = y[:, j * 128:(j + 1) * 128]
                if t == 0:
                    qbuf[j, r0:r0 + M, :] = yj * (0.25 * LOG2E)
                else:
                    buf[j, HALO + r0:HALO + r0 + M, :] = yj
                if i == 0 and t == 2:
                    vbuf[j, 0:HALO, :] = jnp.broadcast_to(yj[0:1, :], (HALO, 128))
            tick(1024, y, 4)
        q_done[0] = i + 1

    accs = {}

    def down(i):
        r0 = i * M
        acc = None
        for c in range(len(KCH) - 1):
            lo, hi = KCH[c], KCH[c + 1]
            wv = wdp.ld(lo, hi, 0, D) if U32 else wd_v[lo:hi, :]
            t = jnp.dot(hb.ld(r0, r0 + M, lo, hi), wv, preferred_element_type=f32)
            tick(-(-(hi - lo) // 128) * 256, t, 4)
            acc = t if acc is None else acc + t
        accs[i] = acc

    def fin(i):
        r0 = i * M
        while sidx[0] < len(sched) and sched[sidx[0]][1] < r0 + M:
            emit_att(sched[sidx[0]][1], None)
            sidx[0] += 1
        t = jnp.dot(ob.ld(r0, r0 + M, 0, D), wop.ld(0, D, 0, D), preferred_element_type=f32)
        x = x_v[r0:r0 + M, :].astype(f32)
        out_v[r0:r0 + M, :] = ((x + accs.pop(i)) + t).astype(out_v.dtype)
        tick(1024, t, 4)
        if not NODMA or i == NB - 1:
            o_copy(i).start()

    qkv(0)
    qkv(1)
    for i in range(NB):
        down(i)
        if i + 2 < NB:
            qkv(i + 2)
        fin(i)
    with scope("waito"):
        for i in range(NB):
            if NODMA and i < NB - 1:
                continue
            o_copy(i).wait()


@jax.jit
def pallas_parallel_sum__sliding_local_dilated__glu_gated_geglu__prompt_kernel(
    A_x, A_wqkv, A_wo, B_x, B_w_gate, B_w_up, B_w_down):
    del B_x
    x = A_x.reshape(S, D)
    anyspec = pl.BlockSpec(memory_space=pl.ANY)
    V = pltpu.VMEM
    pk = (lambda r, c: V((r // 2, c), u32)) if U32 else (lambda r, c: V((r, c), bf))
    small = V((8, 128), u32)
    out = pl.pallas_call(
        _kernel,
        in_specs=[anyspec] * 6,
        out_specs=anyspec,
        out_shape=jax.ShapeDtypeStruct((S, D), A_x.dtype),
        scratch_shapes=[
            V((S, D), bf),
            V((D, 3 * D), bf),
            V((D, D), bf),
            V((DF, D), bf),
            V((DF, D), bf),
            V((DF, D), bf),
            pk(DF, D) if U32 else small,
            pk(DF, D) if U32 else small,
            pk(DF, D) if U32 else small,
            pk(S, D),
            pk(S, DF),
            pk(D, 3 * D),
            pk(D, D),
            V((4, D, 128), f32),
            V((4, S + HALO, 128), f32),
            V((4, S + HALO, 128), f32),
            V((4, S, 128), f32),
            pk(S, D),
            V((S, D), A_x.dtype),
            pltpu.SemaphoreType.DMA((NSEM,)),
        ],
        compiler_params=pltpu.CompilerParams(vmem_limit_bytes=100 * 1024 * 1024, flags=FLAGS),
    )(x, A_wqkv, A_wo, B_w_gate.T, B_w_up.T, B_w_down)
    return out.reshape(1, S, D)
```

```python
import jax
import jax.numpy as jnp
from jax import lax
import jax.experimental.pallas as pl
import jax.experimental.pallas.tpu as pltpu

S, D, DH, W, DIL, DF = 2048, 512, 16, 8, 2, 1376
M = 256
NB = S // M
NIT = 2
NBI = NB // NIT
RI = NBI * M
HALO = 16
RG = 16
UN = 128
CH = (0, 256, 512, 768, 1024, 1376)
ATT0 = (3100, 11000, 19000, 28000)
ATTL = (7900, 8000, 9000, 9000)
LOG2E = 1.4426950408889634
NT = (((1,), (1,)), ((), ()))
bf = jnp.bfloat16
f32 = jnp.float32
u32 = jnp.uint32

NXU = S // UN
SX, SG, SU, SD = 0, NXU, NXU + 6, NXU + 11
SQ = SD + 1
SO = SQ + 1
SOUT = SO + 1
SSLAB = SOUT + NB
NSEM = SSLAB + 4 * NIT


class _Packed:
    def __init__(self, ref):
        self.ref = ref

    def ld(self, r0, r1, c0, c1):
        return pltpu.bitcast(self.ref[r0 // 2:r1 // 2, c0:c1], bf)

    def st(self, r0, r1, c0, c1, val):
        self.ref[r0 // 2:r1 // 2, c0:c1] = pltpu.bitcast(val, u32)


def _perm_tile_cols(wu, j):
    rows = wu.shape[0]
    lane = lax.broadcasted_iota(jnp.int32, (rows, 128), 1)
    hh = lane & 31
    src_tile = hh >> 3
    idx = (hh & 7) * 16 + 4 * j + (lane >> 5)
    acc = None
    for t in range(4):
        g = jnp.take_along_axis(wu[:, t * 128:(t + 1) * 128], idx, axis=1)
        acc = g if acc is None else jnp.where(src_tile == t, g, acc)
    return acc


def _kernel(x_hbm, wqkv_hbm, wo_hbm, wg_hbm, wu_hbm, wd_hbm, out_hbm,
            x_v, wqkv_v, wo_v, wg_v, wu_v, wd_v, wg_p, wu_p, xn_r, h_r, wqkvp_r, wop_r, wof,
            kbuf, vbuf, qbuf, o_r, out_v, sem):
    xn, hb, wqkvp, wop = _Packed(xn_r), _Packed(h_r), _Packed(wqkvp_r), _Packed(wop_r)
    wgp, wup = _Packed(wg_p), _Packed(wu_p)

    def unit(src, dst, base, i):
        sl = pl.ds(i * UN, UN) if isinstance(i, int) else pl.ds(pl.multiple_of(i * UN, UN), UN)
        return pltpu.make_async_copy(src.at[sl], dst.at[sl], sem.at[base + i])

    def start_units(src, dst, base, lo, hi):
        def body(i, c):
            unit(src, dst, base, i).start()
            return c
        lax.fori_loop(lo, hi, body, 0)

    def wait_units(src, dst, base, lo, hi):
        for i in range(lo, hi):
            unit(src, dst, base, i).wait()

    X = (x_hbm, x_v, SX)
    G = (wg_hbm, wg_v, SG)
    U = (wu_hbm, wu_v, SU)
    R0 = CH[2]
    RH = (DF - R0) // 2
    wq_copy = pltpu.make_async_copy(wqkv_hbm, wqkv_v, sem.at[SQ])
    wo_copy = pltpu.make_async_copy(wo_hbm, wo_v, sem.at[SO])
    u_rest = pltpu.make_async_copy(wu_hbm.at[pl.ds(R0, DF - R0)], wu_v.at[pl.ds(R0, DF - R0)], sem.at[SU + 4])
    wd_copy = pltpu.make_async_copy(wd_hbm, wd_v, sem.at[SD])

    def g_rest(i):
        sl = pl.ds(pl.multiple_of(R0 + i * RH, 16), RH)
        return pltpu.make_async_copy(wg_hbm.at[sl], wg_v.at[sl], sem.at[SG + 4 + i])

    start_units(*X, 0, 2)
    start_units(*G, 0, 2)
    start_units(*U, 0, 2)
    start_units(*X, 2, NXU)
    start_units(*G, 2, 4)
    start_units(*U, 2, 4)
    wq_copy.start()
    wo_copy.start()
    lax.fori_loop(0, 2, lambda i, c: (g_rest(i).start(), c)[1], 0)
    u_rest.start()
    wd_copy.start()

    kbuf[:, 0:HALO, :] = jnp.zeros((4, HALO, 128), f32)
    vbuf[:, 0:HALO, :] = jnp.zeros((4, HALO, 128), f32)

    def layernorm(i):
        wait_units(*X, 2 * i, 2 * i + 2)
        x = x_v[i * M:(i + 1) * M, :].astype(f32)
        mu = jnp.mean(x, axis=-1, keepdims=True)
        xc = x - mu
        var = jnp.mean(xc * xc, axis=-1, keepdims=True)
        v = (xc * lax.rsqrt(var + 1e-5)).astype(bf)
        xn.st(i * M, (i + 1) * M, 0, D, v)
        return v

    def getw(raw, pk, i, lo, hi):
        if i == 0:
            v = raw[lo:hi, :]
            pk.st(lo, hi, 0, D, v)
            return v
        return pk.ld(lo, hi, 0, D)

    def gate_up(i, c, xv):
        lo, hi = CH[c], CH[c + 1]
        if i == 0:
            wait_units(*G, lo // UN, hi // UN)
        g = lax.dot_general(xv, getw(wg_v, wgp, i, lo, hi), NT, preferred_element_type=f32)
        if i == 0:
            wait_units(*U, lo // UN, hi // UN)
        u = lax.dot_general(xv, getw(wu_v, wup, i, lo, hi), NT, preferred_element_type=f32)
        hb.st(i * M, (i + 1) * M, lo, hi, (jax.nn.gelu(g, approximate=True) * u).astype(bf))

    def perm_qkv(t):
        wu = pltpu.bitcast(wqkv_v[:, t * 512:(t + 1) * 512], u32)
        for j in range(4):
            c0 = t * 512 + j * 128
            wqkvp.st(0, D, c0, c0 + 128, pltpu.bitcast(_perm_tile_cols(wu, j), bf))

    def perm_wo():
        for j in range(4):
            wof[j] = wo_v[:, j * 128:(j + 1) * 128].astype(f32)
        for d in range(DH):
            for j in range(4):
                wop.st(d * 32, (d + 1) * 32, j * 128, (j + 1) * 128,
                       wof[j, pl.ds(d, 32, stride=16), :].astype(bf))

    for c in range(2):
        for i in range(NB):
            xv = layernorm(i) if c == 0 else xn.ld(i * M, (i + 1) * M, 0, D)
            gate_up(i, c, xv)
            if c == 1 and i == 0:
                wq_copy.wait()
                wo_copy.wait()
                for t in range(3):
                    perm_qkv(t)
    lax.fori_loop(0, 2, lambda i, c: (g_rest(i).wait(), c)[1], 0)
    u_rest.wait()
    wd_copy.wait()

    def o_copy(i):
        return pltpu.make_async_copy(out_v.at[pl.ds(i * M, M)], out_hbm.at[pl.ds(i * M, M)], sem.at[SOUT + i])

    def slab_copy(it, n):
        r = (it + 1) * RI - M
        sl = pl.ds(r, M) if isinstance(it, int) else pl.ds(pl.multiple_of(r, M), M)
        cs = pl.ds(n * 128, 128)
        return pltpu.make_async_copy(out_v.at[sl, cs], out_hbm.at[sl, cs], sem.at[SSLAB + it * 4 + n])

    def phase2(it, carry):
        base = pl.multiple_of(it * RI, RI)
        hbase = pl.multiple_of(it * (RI // 2), RI // 2)
        xn_i = _Packed(xn_r.at[pl.ds(hbase, RI // 2)])
        hb_i = _Packed(h_r.at[pl.ds(hbase, RI // 2)])
        ob_i = _Packed(o_r.at[pl.ds(hbase, RI // 2)])
        kb = kbuf.at[:, pl.ds(base, RI + HALO), :]
        vb = vbuf.at[:, pl.ds(base, RI + HALO), :]
        x_i = x_v.at[pl.ds(base, RI)]
        out_i = out_v.at[pl.ds(base, RI)]

        def att(g0, gate):
            q = [qbuf[j, g0:g0 + RG, :] for j in range(4)]
            if gate is not None:
                z = gate - gate
                z = jnp.where(z == 0.0, z, 0.0)
                z = jnp.concatenate([z] * (RG // 8), axis=0)
                q = [qq + z for qq in q]
            ls = []
            for w in range(W):
                off = HALO + g0 - DIL * w
                s = None
                for j in range(4):
                    p = q[j] * kb[j, off:off + RG, :]
                    s = p if s is None else s + p
                s = s + pltpu.roll(s, 64, 1)
                s = s + pltpu.roll(s, 32, 1)
                if g0 < DIL * w:
                    pos = base + g0 + lax.broadcasted_iota(jnp.int32, (RG, 128), 0)
                    s = jnp.where(pos >= DIL * w, s, -1e9 * LOG2E)
                ls.append(s)
            m = ls[0]
            for w in range(1, W):
                m = jnp.maximum(m, ls[w])
            es = [jnp.exp2(l - m) for l in ls]
            den = es[0]
            for w in range(1, W):
                den = den + es[w]
            inv = pl.reciprocal(den, approx=True)
            inv = inv * (2.0 - den * inv)
            for j in range(4):
                o = None
                for w in range(W):
                    off = HALO + g0 - DIL * w
                    t = es[w] * vb[j, off:off + RG, :]
                    o = t if o is None else o + t
                ob_i.st(g0, g0 + RG, j * 128, (j + 1) * 128, (o * inv).astype(bf))

        sched = []
        for i in range(NBI):
            n = M // RG
            for c in range(n):
                sched.append((ATT0[i] + ATTL[i] * c // n, i * M + c * RG))
        st = {"now": 0, "next": 0, "qrows": 0}

        def tick(cycles, val, nparts):
            for p in range(nparts):
                for hrow in range(2):
                    t = st["now"] + cycles * (2 * p + hrow) // (2 * nparts)
                    gv = val[hrow * 128:hrow * 128 + 8, p * 128:(p + 1) * 128]
                    while (st["next"] < len(sched) and sched[st["next"]][0] <= t
                           and sched[st["next"]][1] < st["qrows"]):
                        att(sched[st["next"]][1], gv)
                        st["next"] += 1
            st["now"] += cycles

        def qkv(i):
            r0 = i * M
            xv = xn_i.ld(r0, r0 + M, 0, D)
            for t, buf in ((1, kb), (2, vb), (0, None)):
                y = jnp.dot(xv, wqkvp.ld(0, D, t * 512, (t + 1) * 512), preferred_element_type=f32)
                for j in range(4):
                    yj = y[:, j * 128:(j + 1) * 128]
                    if t == 0:
                        qbuf[j, r0:r0 + M, :] = yj * (0.25 * LOG2E)
                    else:
                        buf[j, HALO + r0:HALO + r0 + M, :] = yj
                    if i == 0 and t == 2:
                        v0 = jnp.broadcast_to(yj[0:1, :], (HALO, 128))
                        vb[j, 0:HALO, :] = jnp.where(it == 0, v0, vb[j, 0:HALO, :])
                tick(1024, y, 4)
            st["qrows"] = r0 + M

        def gate_up_rest(i):
            r0 = i * M
            xv = xn_i.ld(r0, r0 + M, 0, D)
            for c in range(2, len(CH) - 1):
                lo, hi = CH[c], CH[c + 1]
                nt = -(-(hi - lo) // 128)
                g = lax.dot_general(xv, wg_v[lo:hi, :], NT, preferred_element_type=f32)
                tick(nt * 256, g, (hi - lo) // 128)
                u = lax.dot_general(xv, wu_v[lo:hi, :], NT, preferred_element_type=f32)
                tick(nt * 256, u, (hi - lo) // 128)
                hb_i.st(r0, r0 + M, lo, hi, (jax.nn.gelu(g, approximate=True) * u).astype(bf))

        def down(i):
            r0 = i * M
            acc = None
            for c in range(len(CH) - 1):
                lo, hi = CH[c], CH[c + 1]
                t = jnp.dot(hb_i.ld(r0, r0 + M, lo, hi), wd_v[lo:hi, :], preferred_element_type=f32)
                tick(-(-(hi - lo) // 128) * 256, t, 4)
                acc = t if acc is None else acc + t
            return acc

        def finish(i, acc):
            r0 = i * M
            while st["next"] < len(sched) and sched[st["next"]][1] < r0 + M:
                att(sched[st["next"]][1], None)
                st["next"] += 1
            ov = ob_i.ld(r0, r0 + M, 0, D)
            if i == NBI - 1:
                for n in range(4):
                    cs = slice(n * 128, (n + 1) * 128)
                    t = jnp.dot(ov, wop.ld(0, D, n * 128, (n + 1) * 128), preferred_element_type=f32)
                    out_i[r0:r0 + M, cs] = (
                        (x_i[r0:r0 + M, cs].astype(f32) + acc[:, cs]) + t).astype(out_v.dtype)
                    slab_copy(it, n).start()
                return
            t = jnp.dot(ov, wop.ld(0, D, 0, D), preferred_element_type=f32)
            out_i[r0:r0 + M, :] = ((x_i[r0:r0 + M, :].astype(f32) + acc) + t).astype(out_v.dtype)
            tick(1024, t, 4)
            gi = it * NBI + i
            sl = pl.ds(pl.multiple_of(gi * M, M), M)
            pltpu.make_async_copy(out_v.at[sl], out_hbm.at[sl], sem.at[SOUT + gi]).start()

        perm_wo()
        qkv(0)
        gate_up_rest(0)
        qkv(1)
        gate_up_rest(1)
        for i in range(NBI):
            acc = down(i)
            if i + 2 < NBI:
                qkv(i + 2)
                gate_up_rest(i + 2)
            finish(i, acc)
        return carry

    lax.fori_loop(0, NIT, phase2, 0)
    for i in range(NB):
        if (i + 1) % NBI == 0:
            for n in range(4):
                slab_copy(i // NBI, n).wait()
        else:
            o_copy(i).wait()


@jax.jit
def pallas_parallel_sum__sliding_local_dilated__glu_gated_geglu__prompt_kernel(
    A_x: jax.Array,
    A_wqkv: jax.Array,
    A_wo: jax.Array,
    B_x: jax.Array,
    B_w_gate: jax.Array,
    B_w_up: jax.Array,
    B_w_down: jax.Array,
):
    del B_x
    anyspec = pl.BlockSpec(memory_space=pl.ANY)
    V = pltpu.VMEM
    packed = lambda r, c: V((r // 2, c), u32)
    out = pl.pallas_call(
        _kernel,
        in_specs=[anyspec] * 6,
        out_specs=anyspec,
        out_shape=jax.ShapeDtypeStruct((S, D), A_x.dtype),
        scratch_shapes=[
            V((S, D), bf),
            V((D, 3 * D), bf),
            V((D, D), bf),
            V((DF, D), bf),
            V((DF, D), bf),
            V((DF, D), bf),
            packed(CH[2], D),
            packed(CH[2], D),
            packed(S, D),
            packed(S, DF),
            packed(D, 3 * D),
            packed(D, D),
            V((4, D, 128), f32),
            V((4, S + HALO, 128), f32),
            V((4, S + HALO, 128), f32),
            V((4, RI, 128), f32),
            packed(S, D),
            V((S, D), A_x.dtype),
            pltpu.SemaphoreType.DMA((NSEM,)),
        ],
        compiler_params=pltpu.CompilerParams(
            vmem_limit_bytes=100 * 1024 * 1024,
            flags={"XLA_TPU_RESCHEDULE_DMA_DONES": True},
            disable_semaphore_checks=True,
        ),
    )(A_x.reshape(S, D), A_wqkv, A_wo, B_w_gate.T, B_w_up.T, B_w_down)
    return out.reshape(1, S, D)
```
